```python
import jax
import jax.numpy as jnp

def _softmax(x, axis=-1):
    return jax.nn.softmax(x, axis=axis)

def _gelu(x):
    return jax.nn.gelu(x, approximate=True)

def _silu(x):
    return jax.nn.silu(x)

def _sigmoid(x):
    return jax.nn.sigmoid(x)

def _layernorm(x, axis=-1, eps=1e-05):
    m = jnp.mean(x, axis=axis, keepdims=True)
    v = jnp.var(x, axis=axis, keepdims=True)
    return (x - m) / jnp.sqrt(v + eps)

def _scatter_add(tgt, idx, src, axis=0):
    return tgt.at[idx].add(src)

def _segment_sum(src, seg, n):
    return jax.ops.segment_sum(src, seg, n)

class _Rng:

    def __init__(self, key):
        self._k = key

    def _next(self):
        self._k, sub = jax.random.split(self._k)
        return sub

    def normal(self, shape):
        return jax.random.normal(self._next(), shape, dtype=jnp.bfloat16)

    def randint(self, lo, hi, shape):
        return jax.random.randint(self._next(), shape, lo, hi, dtype=jnp.int32)

    def uniform(self, shape, lo=0.0, hi=1.0):
        return jax.random.uniform(self._next(), shape, jnp.bfloat16, lo, hi)

    def permutation(self, n):
        return jax.random.permutation(self._next(), n)
kernel_name = 'adaLN_cond__grouped_kv_mqa__mixer_token_mlp__prompt'

def _fwd_setup_inputs():
    _rng = _Rng(jax.random.key(int.from_bytes(__import__("os").urandom(4), "little")))
    _w = lambda a: (lambda t: t.astype(jnp.bfloat16) if jnp.issubdtype(t.dtype, jnp.floating) else t)(jnp.asarray(a))

    def _A_setup():
        B, S, D, H = (1, 2048, 512, 32)
        Dh = D // H
        return {'x': _w((lambda *s: _rng.normal(s) * 0.05)(B, S, D)), 'wq': _w((lambda *s: _rng.normal(s) * 0.05)(D, H * Dh)), 'wk': _w((lambda *s: _rng.normal(s) * 0.05)(D, Dh)), 'wv': _w((lambda *s: _rng.normal(s) * 0.05)(D, Dh)), 'wo': _w((lambda *s: _rng.normal(s) * 0.05)(H * Dh, D))}
    _A_in = _A_setup()

    def _B_setup():
        B, S, D, F = (1, 2048, 512, 1376)
        return {'x': _w((lambda *s: _rng.normal(s) * 0.05)(B, S, D)), 'w1': _w((lambda *s: _rng.normal(s) * 0.05)(S, F) * S ** (-0.5)), 'b1': _w((lambda *s: _rng.normal(s) * 0.05)(F) * 0.02), 'w2': _w((lambda *s: _rng.normal(s) * 0.05)(F, S) * F ** (-0.5)), 'b2': _w((lambda *s: _rng.normal(s) * 0.05)(S) * 0.02)}
    _B_in = _B_setup()
    return {'A_x': _A_in['x'], 'A_wq': _A_in['wq'], 'A_wk': _A_in['wk'], 'A_wv': _A_in['wv'], 'A_wo': _A_in['wo'], 'B_x': _B_in['x'], 'B_w1': _B_in['w1'], 'B_b1': _B_in['b1'], 'B_w2': _B_in['w2'], 'B_b2': _B_in['b2'], 'c': _w((lambda *s: _rng.normal(s) * 0.05)(1, 512)), 'w_mod': _w((lambda *s: _rng.normal(s) * 0.05)(512, 6 * 512) * 512 ** (-0.5))}

def _fwd_reference(A_x, A_wq, A_wk, A_wv, A_wo, B_x, B_w1, B_b1, B_w2, B_b2, c, w_mod):

    def _A_ref(x, wq, wk, wv, wo):
        B, S, D = x.shape
        H = 32
        Dh = D // H
        q = (lambda x, *d: x.transpose(*d))((x @ wq).reshape(B, S, H, Dh), 0, 2, 1, 3)
        k = x @ wk
        v = x @ wv
        scores = jnp.einsum('bhqd,bkd->bhqk', q, k) * Dh ** (-0.5)
        p = _softmax(scores, axis=-1)
        o = jnp.einsum('bhqk,bkd->bhqd', p, v)
        return (lambda x, *d: x.transpose(*d))(o, 0, 2, 1, 3).reshape(B, S, H * Dh) @ wo

    def _B_ref(x, w1, b1, w2, b2):
        B, S, D = x.shape
        h = _layernorm(x, axis=-1)
        u = jnp.einsum('bsd,sf->bdf', h, w1) + b1
        u = _gelu(u)
        y = jnp.einsum('bdf,fs->bds', u, w2) + b2
        return (lambda x, *d: x.transpose(*d))(y, 0, 2, 1)
    x = A_x
    mod = (_silu(c) @ w_mod).reshape(c.shape[0], 6, 1, -1)
    sa, ca, ga, sb, cb, gb = (mod[:, 0].copy(), mod[:, 1].copy(), mod[:, 2].copy(), mod[:, 3].copy(), mod[:, 4].copy(), mod[:, 5].copy())
    h = _layernorm(x, axis=-1) * (1 + ca) + sa
    x = x + ga * _A_ref(h, A_wq, A_wk, A_wv, A_wo)
    h = _layernorm(x, axis=-1) * (1 + cb) + sb
    x = x + gb * _B_ref(h, B_w1, B_b1, B_w2, B_b2)
    return x

def setup_inputs():
    _inp = _fwd_setup_inputs()
    _gk = jax.random.fold_in(jax.random.key(int.from_bytes(__import__("os").urandom(4), "little")), 2 ** 31 - 1)
    _shapes = [[1, 2048, 512]]
    _dtypes = ['bfloat16']
    _gks = jax.random.split(_gk, len(_shapes))
    _gs = [jax.random.normal(k, s, dtype=jnp.dtype(d)) * 0.05 for k, s, d in zip(_gks, _shapes, _dtypes)]
    _inp['grad_out'] = _gs[0]
    return _inp

def reference(A_x, A_wq, A_wk, A_wv, A_wo, B_w1, B_b1, B_w2, B_b2, c, w_mod, B_x, grad_out):
    _const = dict(B_x=B_x)

    def _f(*_d):
        return _fwd_reference(**{'A_x': _d[0], 'A_wq': _d[1], 'A_wk': _d[2], 'A_wv': _d[3], 'A_wo': _d[4], 'B_w1': _d[5], 'B_b1': _d[6], 'B_w2': _d[7], 'B_b2': _d[8], 'c': _d[9], 'w_mod': _d[10], **_const})
    _out, _vjp = jax.vjp(_f, A_x, A_wq, A_wk, A_wv, A_wo, B_w1, B_b1, B_w2, B_b2, c, w_mod)
    _grads = _vjp(grad_out)
    _out0 = jnp.asarray(_out)
    return (_out0, *[jnp.asarray(_g) for _g in _grads])
```

```python
import functools
import math

import jax
import jax.numpy as jnp
from jax import lax
import jax.experimental.pallas as pl
import jax.experimental.pallas.tpu as pltpu

F32, BF16, U32 = jnp.float32, jnp.bfloat16, jnp.uint32

S, D, H, DH, F = 2048, 512, 32, 16, 1376
EPS = 1e-5
LOG2E = math.log2(math.e)
QSCALE = DH ** -0.5 * LOG2E

BQ = 512
LT = BQ // 128
KC = 128
KV = 16
KM = KC - KV
NK = S // KC
LAG = 2
NP = H * S // (2 * BQ)
UP = 4
NI = NP // UP
FWD_PARTS = (3, 2, 5, 5, 3, 6, 3, 5)
REDO_PARTS = (4, 4, 8, 4, 4, 8)
BWD_PARTS = (2, 1, 5, 2, 3, 4, 4, 0, 3, 3, 5)
N_RING = 5
N_RES = 56
PAGES = LT * NK * KM // 512
REDO_A = NP - N_RES

SAFE = 40

TC = 512
NS = S // 128
ND = D // 128
FC = 256
F_CHUNKS = [(F - F % FC, F % FC)] + [(f, FC) for f in range(0, F - F % FC, FC)]

ALL = slice(None)


def _dot(a, b):
    return jnp.dot(a, b, preferred_element_type=F32)


def _dot_nt(a, b):
    return lax.dot_general(a, b, (((1,), (1,)), ((), ())), preferred_element_type=F32)


def _words(x):
    return pltpu.bitcast(x, U32)


def _ld(ref, *idx):
    return pltpu.bitcast(ref[idx], BF16)


def _pk(x):
    return _words(x.astype(BF16))


def _span(i, n, size=None):
    return pl.ds(i * n if isinstance(i, int) else pl.multiple_of(i * n, n), size or n)


def _lanes(j):
    return slice(j * 128, (j + 1) * 128)


def _col(row):
    return jnp.broadcast_to(row, (128, row.shape[1])).T


def _row_total(acc):
    return jnp.sum(acc.T, axis=0, keepdims=True)


def _after(never, words, reg):
    if reg is None:
        return words
    first = jnp.where(never, reg if reg.dtype == U32 else _words(reg), words[:, :128])
    return first if words.shape[1] == 128 else jnp.concatenate([first, words[:, 128:]], axis=1)


class _Pacer:
    def __init__(self, never):
        self.never, self.gate, self.jobs = never, None, {True: [], False: []}

    def add(self, job, pieces, begin, end, ahead=False):
        self.jobs[ahead].append([job, begin, (end - begin) / pieces])

    def now(self, row, rows):
        reg = jnp.broadcast_to(row, (8, 128))
        if self.gate is not None:
            reg = jnp.where(self.never, self.gate, reg)
        return jnp.concatenate([reg] * ((rows.stop - rows.start) // 8), axis=0)

    def _advance(self, jobs, before):
        for item in list(jobs):
            while item[1] < 1:
                before(item[1])
                reg = next(item[0], False)
                if reg is False:
                    jobs.remove(item)
                    break
                yield item[1], reg
                item[1] += item[2]
            item[1] -= 1

    def drain(self):
        for job, _, _ in self.jobs[True] + self.jobs[False]:
            list(job)
        self.jobs = {True: [], False: []}

    def dot(self, words, rhs, dot=_dot):
        slots = [words[r:r + 8] for r in range(0, words.shape[0], 8)]
        for when, reg in self._advance(self.jobs[True], lambda when: None):
            i = int(when * len(slots))
            slots[i] = _after(self.never, slots[i], reg)
        out = dot(pltpu.bitcast(jnp.concatenate(slots, axis=0), BF16), rhs)

        def before(when):
            r = int(when * len(slots)) * 16
            self.gate = out[r:r + 8]

        list(self._advance(self.jobs[False], before))
        self.gate = None
        return out


def _row_groups(n):
    return [(slice(r, r + 8 * n), slice(r // 2, r // 2 + 4 * n)) for r in range(0, D, 8 * n)]


def _mean(x):
    return jnp.sum(x, axis=0, keepdims=True) * (1.0 / D)


def _means(n, fn):
    acc = None
    for rows, words in _row_groups(n):
        part = [jnp.sum(x.reshape(n, 8, 128), axis=0) for x in fn(rows, words)]
        acc = part if acc is None else [a + b for a, b in zip(acc, part)]
        yield acc[0]
    return [_mean(a) for a in acc]


def _rstd(n, centered):
    var, = yield from _means(n, lambda rows, words: [jnp.square(centered(rows, words))])
    return lax.rsqrt(var + EPS)


def _gelu_and_grad(u):
    c0, c1 = math.sqrt(2.0 / math.pi), 0.044715
    u2 = u * u
    t = jnp.tanh(u * (c0 + (c0 * c1) * u2))
    cdf = 0.5 + 0.5 * t
    grad = cdf + (0.5 * u) * (1.0 - t * t) * (c0 + (3.0 * c0 * c1) * u2)
    return u * cdf, grad


def _head(ref, h, n):
    return jnp.concatenate([ref[n * LT + j, _span(h, DH), :] for j in range(LT)], axis=1)


def _set_head(ref, h, n, x):
    for j in range(LT):
        ref[n * LT + j, _span(h, DH), :] = x[:, _lanes(j)].astype(BF16)


def _strips(ref, first, n, rows=ALL):
    return jnp.concatenate([ref[first + j, rows, :] for j in range(n)], axis=1)


def _put(ref, idx, rows, x):
    for j in range(LT):
        ref[idx, j, rows, :] = x[:, _lanes(j)].astype(BF16)


def _get(ref, idx, rows):
    return jnp.concatenate([ref[idx, j, rows, :] for j in range(LT)], axis=1)


def _fill_table(table_ref, words_ref, t, first, skip=0):
    x = _ld(words_ref, _span(t, KC // 2, (skip + KV) // 2), ALL)[skip:].astype(F32)
    for r in range(KV // 8):
        for d in range(0, DH, 4):
            regs = _words(jnp.concatenate([jnp.broadcast_to(x[r * 8:(r + 1) * 8, e:e + 1], (8, 128))
                                           for e in range(first + d, first + d + 4)], axis=0))
            table_ref[t, pl.ds((r * DH + d) * 8, 32), :] = regs
            yield regs[-8:]


def _vpu_rows(table_ref, t, q_ref, sizes, init=None):
    rows, progress = [], []
    for j in range(LT):
        keys = lax.split(pltpu.bitcast(table_ref[t], F32).reshape(KV // 8, DH, 8, 128), (1,) * DH, axis=1)
        q = [jnp.broadcast_to(q_ref[d:d + 1, _lanes(j)], (1, 1, 8, 128)) for d in range(DH)]
        acc = None if init is None else init[j]
        for d in range(0, DH, 2):
            pair = keys[d] * q[d] + keys[d + 1] * q[d + 1]
            acc = pair if acc is None else acc + pair
            progress.append(acc)
        rows.append(acc.reshape(KV, 128))
    done, parts = 0, []
    for size in sizes:
        ends = [i for i in range(done, done + size) if (i + 1) % (DH // 2) == 0 or i + 1 == done + size]
        part = functools.reduce(jnp.add, [progress[i] if init else progress[i][-1:] for i in ends]) if ends else None
        parts.append(jnp.sum(part, axis=(0, 1)) if ends else None)
        done += size
    return jnp.concatenate(rows, axis=1), parts


def _mxu_keys(never, words_ref, t, parts):
    words = words_ref[(t + 1) * KC // 2 - 8 * len(parts):(t + 1) * KC // 2, :]
    regs = [_after(never, words[i * 8:(i + 1) * 8], part) for i, part in enumerate(parts)]
    return pltpu.bitcast(jnp.concatenate(regs, axis=0), BF16)


def _blocks(i):
    return [(2 * k + b, i * UP + k, i * (UP // 2) + k // 2, 2 * (k % 2) + b, b) for b in (1, 0) for k in range(UP)]


def _ring(p):
    return lax.rem(p + N_RING - NP % N_RING, N_RING)


def _ring_back(k):
    return (2, 1, 0, 3)[k]


def _a_slot(p):
    spare = jnp.where(p & (2 * UP - 1) == UP, 2 * UP, UP + (p & (UP - 1)))
    return jnp.where(p < REDO_A, spare, p - REDO_A)


def _start(copies):
    for src, dst, sem in copies:
        pltpu.make_async_copy(src, dst, sem).start()


def _wait(copies):
    for src, dst, sem in copies:
        pltpu.make_async_copy(src, dst, sem).wait()


def _copies(pairs, sem, out=False):
    return [(b, a, sem) if out else (a, b, sem) for a, b in pairs]


def _kernel(x_hbm, wq_hbm, wkt_hbm, wvt_hbm, wo_hbm, w1t_hbm, b1_hbm, w2_hbm, b2_hbm, c_hbm, wmod_hbm, g_hbm,
            out_hbm, dx_hbm, dwq_hbm, dwkt_hbm, dwvt_hbm, dwo_hbm, dw1t_hbm, db1_hbm, dw2_hbm, db2_hbm,
            dc_hbm, dwmod_hbm, p_hbm,
            p_s, xt_s, qt_s, ot_s, gt_s, h_s, k_s, kvt_s, wo_s, wkv_s, b1_s, b2_s, c_s, m_s, l_s,
            mod_s, dmod_s, st_s, q32_s, lag_s, top_s, zero_s, p_sem, b_sem, g_sem):
    n_tc = S // TC

    def token_copies(hbm, i, ref, first, sem, out=False):
        return _copies([(hbm.at[0, _span(i, TC), pl.ds(j * 128, 128)], ref.at[first + j]) for j in range(ND)],
                       sem, out)

    def staged(hbm, i, slot, sem, out=False):
        return token_copies(hbm, i, p_s, slot * PAGES + ND * i, sem, out)

    def staged_tile(slot, s, d):
        return slot * PAGES + (s >> 2) * ND + d, _span(s & 3, 128)

    def p_tile(slot, t, j):
        return pl.ds(slot * PAGES + (t >> 3) * (KM // 16), KM // 16), _span((t & 7) * LT + j, 16)

    def p_put(slot, t, e):
        for j in range(LT):
            p_s[p_tile(slot, t, j)] = e[:, _lanes(j)].reshape(KM // 16, 16, 128).astype(BF16)

    def square_copies(hbm, sem, out=False):
        return _copies([(hbm.at[:, pl.ds(j * 128, 128)], wo_s.at[0, j]) for j in range(ND)], sem, out)

    def transpose_x(slot, s, rows, words):
        tile = p_s[staged_tile(slot, s, rows.start // 128)].T
        xt_s[s, words] = _words(tile)
        return tile

    def acc_at(n, rows):
        if rows.stop - rows.start == D:
            return (slice(2 * n, 2 * n + 2),)
        strip, row = divmod(rows.start, D // 2)
        return 2 * n + strip, slice(row, row + rows.stop - rows.start)

    def acc_get(n, rows=slice(0, D)):
        return pltpu.bitcast(h_s[acc_at(n, rows)].reshape(rows.stop - rows.start, 128), F32)

    def acc_set(n, x, rows=slice(0, D)):
        h_s[acc_at(n, rows)] = _words(x).reshape(h_s.at[acc_at(n, rows)].shape)

    def acc_add(n, x, rows=slice(0, D)):
        acc_set(n, acc_get(n, rows) + x, rows)

    def mod(i):
        return mod_s[:, i * D:(i + 1) * D]

    def silu_c():
        c_in = c_s[...].astype(F32)
        return (c_in * jax.nn.sigmoid(c_in)).astype(BF16)

    def never():
        return zero_s[...] > 0

    def p_store(p):
        return [(p_s.at[pl.ds((N_RES + _ring(p)) * PAGES, PAGES)], p_hbm.at[p], p_sem.at[_ring(p)])]

    def p_load(i, k):
        return [(p_hbm.at[i * UP + k], p_s.at[pl.ds((N_RES + _ring_back(k)) * PAGES, PAGES)], p_sem.at[_ring_back(k)])]

    def free_ring(i):
        for k in range(UP):
            pl.when(i * UP + k >= N_RING)(lambda p=i * UP + k - N_RING: _wait(p_store(p)))

    def scores(q, t):
        return _dot(_ld(k_s, _span(t, KC // 2), ALL)[:, :DH], q)

    def carried(st):
        return [(st, NK - LAG + u, _get(lag_s, u, ALL)) for u in range(LAG)]

    biases = [(b1_hbm, b1_s, b_sem.at[0]), (b2_hbm, b2_s, b_sem.at[1])]
    bias_grads = [(b1_s, db1_hbm, b_sem.at[0]), (b2_s, db2_hbm, b_sem.at[1])]

    def g_in(i):
        return staged(g_hbm, i, N_RES - 2, g_sem.at[i])

    def prologue(wmod_buf, wq_buf, wt_s, col_s, sem):
        x_in = [staged(x_hbm, i, 0, sem.at[0, i]) for i in range(n_tc)]
        wmod_a = [(c_hbm, c_s, sem.at[1, 0]),
                  (wmod_hbm.at[:, pl.ds(0, 2 * D)], wmod_buf.at[:, pl.ds(0, 2 * D)], sem.at[1, 0])]
        wmod_b = [(wmod_hbm.at[:, pl.ds(2 * D, 4 * D)], wmod_buf.at[:, pl.ds(2 * D, 4 * D)], sem.at[1, 1])]
        w_in = _copies([(wq_hbm, wq_buf), (wkt_hbm, wkv_s.at[pl.ds(0, DH)]), (wvt_hbm, wkv_s.at[pl.ds(DH, DH)])],
                       sem.at[1, 2])
        wo_in = square_copies(wo_hbm, sem.at[1, 3])
        _start(wmod_a + x_in[0])
        zero_s[...] = jnp.zeros(zero_s.shape, F32)
        m_s[...] = jnp.zeros(m_s.shape, F32)
        lag_s[...] = jnp.zeros(lag_s.shape, BF16)
        _wait(wmod_a)
        _start(w_in + x_in[1])
        silu_rows = jnp.broadcast_to(silu_c(), (16, D))
        mod_s[:, 0:2 * D] = _dot(silu_rows, wmod_buf[:, 0:2 * D])[0:1]
        col_s[0] = _col(mod(0))
        col_s[1] = _col(1.0 + mod(1))
        pace, ready = _Pacer(never()), {}

        def center(s):
            st_s[0, :, _lanes(s)], = yield from _means(16, lambda *r: [transpose_x(0, s, *r).astype(F32)])

        def normalize(s):
            mean = st_s[0, :, _lanes(s)]
            rstd = yield from _rstd(8, lambda rows, words: _ld(xt_s, s, words).astype(F32) - pace.now(mean, rows))
            st_s[1, :, _lanes(s)] = rstd
            h1 = []
            for rows, words in _row_groups(8):
                n1 = (_ld(xt_s, s, words).astype(F32) - mean) * pace.now(rstd, rows)
                h1.append(n1 * col_s[1, rows] + col_s[0, rows])
                yield
            ready[s] = jnp.concatenate(h1, axis=0).astype(BF16)

        def transpose_wo():
            for j in range(ND):
                for r in range(j + 1):
                    tiles = {(a, b): wo_s[0, a, _lanes(b), :].astype(F32).T for a, b in ((j, r), (r, j))}
                    for (a, b), tile in tiles.items():
                        wo_s[0, b, _lanes(a), :] = tile.astype(BF16)
                        yield tile[-8:]

        _wait(x_in[0])
        for s in range(4):
            list(center(s))
        for s in range(3):
            list(normalize(s))
        _wait(w_in)
        _start(x_in[2])
        wt_s[0:D // 2, :] = _words(wq_buf[...].T)
        wt_s[D // 2:D // 2 + DH, :] = _words(wkv_s[...])
        for s in range(NS):
            if s == 1:
                _wait(x_in[1])
                _start(x_in[3] + wo_in)
            elif s == 4:
                _wait(x_in[2])
                _start(wmod_b + biases)
            elif s == 8:
                _wait(x_in[3] + wo_in)
                _start(sum((g_in(i) for i in range(n_tc)), []))
                pace.add(transpose_wo(), 16, 0.4, 4.4, ahead=True)
            for u in {0: [], 1: [4, 5]}.get(s, [s + 4]):
                if u < NS:
                    pace.add(center(u), 4, 0.3, 1.0, ahead=True)
            for u in {1: [], 2: [4, 5]}.get(s, [s + 3]):
                if u < NS:
                    pace.add(normalize(u), 16, 0.0, 0.95)
            for u in range(4 * (s - 12), min(4 * (s - 11), NS - 2)) if s >= 12 else ():
                pace.add(_fill_table(h_s, k_s, u, 0), 8, 0.4, 1.0, ahead=True)
            qkv = pace.dot(wt_s[...], ready.pop(s))
            qt_s[s] = (qkv[0:D] * QSCALE).astype(BF16)
            kvt_s[:, _lanes(s)] = _pk(qkv[D:])
            k_s[_span(s, 64), :] = _words(
                jnp.concatenate([qkv[D:], jnp.zeros((128 - 2 * DH, 128), F32)], axis=0).astype(BF16).T)
        pace.drain()
        _wait(wmod_b)
        mod_s[:, 2 * D:6 * D] = _dot(silu_rows, wmod_buf[:, 2 * D:6 * D])[0:1]
        for u in range(NS - 2, NS):
            list(_fill_table(h_s, k_s, u, 0))

    pl.run_scoped(prologue, pltpu.VMEM((D, 6 * D), BF16), pltpu.VMEM((D, D), BF16),
                  pltpu.VMEM((D // 2 + DH, D), U32), pltpu.VMEM((2, D, 128), F32), pltpu.SemaphoreType.DMA((2, 4)))

    def forward():
        def use(st, t, e, l=None, part=None):
            vt = kvt_s[8:16, _lanes(t)]
            if part is not None:
                if l is not None and t % 2:
                    part = part + ((l[:, _lanes(0)] + l[:, _lanes(1)]) + (l[:, _lanes(2)] + l[:, _lanes(3)]))
                vt = _after(never(), vt, part)
            st[0] = st[0] + _dot(pltpu.bitcast(vt, BF16), e)
            if t == NK - 1:
                _, l, h, n = st
                l = jnp.sum(l, axis=0, keepdims=True)
                inv = pl.reciprocal(l, approx=True)
                inv = inv * (2.0 - l * inv)
                l_s[h, :, _span(n, BQ)] = inv
                _set_head(ot_s, h, n, st[0] * inv)

        def heads(i, prev):
            free_ring(i)

            pl.when(i & 3 == 0)(lambda: _wait(g_in(i >> 2)))
            for d in range(ND):
                gt_s[_span(d, 64), _span(i, 128)] = _words(p_s[staged_tile(N_RES - 2, i, d)].T)

            mask = never()
            qs = [_head(qt_s, h, n) for _, _, h, n, _ in _blocks(i)]
            for pos, q in enumerate(qs):
                q32_s[pos] = q.astype(F32)
            pending = carried([*prev, *_blocks(jnp.maximum(i - 1, 0))[-1][2:4]])
            for pos, (_, p, h, n, b) in enumerate(_blocks(i)):
                slot = N_RES + _ring(p) if b else _a_slot(p)
                st = [jnp.zeros((DH, BQ), F32), jnp.zeros((8, BQ), F32), h, n]
                for t in range(NK):
                    rows, parts = _vpu_rows(h_s, t, q32_s.at[pos], FWD_PARTS)
                    free = 3 if pos == t == 0 else 0
                    keys = _mxu_keys(mask, k_s, t, [None] * free + parts[free:-1])
                    e = jnp.exp2(jnp.concatenate([rows, _dot(keys[:, :DH], qs[pos])], axis=0))
                    st[1] = st[1] + jnp.sum(e.reshape(KC // 8, 8, BQ), axis=0)
                    p_put(slot, t, e[KV:])
                    if pos == 2 * UP - 1 and t >= NK - LAG:
                        _put(lag_s, t - (NK - LAG), ALL, e)
                    else:
                        pending.append((st, t, e.astype(BF16), st[1]))
                    use(*pending.pop(0), part=parts[-1])
                if pos < UP - 1:
                    _start(p_store(p))
                elif b:
                    pl.when(p < NP - 1)(lambda p=p: _start(p_store(p)))
            return st[0], st[1]

        last = lax.fori_loop(0, NI, heads, (jnp.zeros((DH, BQ), F32), jnp.ones((8, BQ), F32)))
        for item in carried([*last, *_blocks(NI - 1)[-1][2:4]]):
            use(*item)

    forward()
    safe = jnp.ones((1, S), F32)
    for h in range(H):
        inv = l_s[h]
        safe = jnp.where(inv >= 2.0 ** -SAFE, jnp.where(inv <= 2.0 ** SAFE, safe, 0.0), 0.0)
    no_shift = jnp.min(safe) > 0

    @pl.when(jnp.logical_not(no_shift))
    def _():
        def block(j, carry):
            p, b = j >> 1, j & 1
            h, n = p >> 1, j & 3
            pl.when(j & (2 * UP - 1) == 0)(lambda: free_ring(lax.div(p, UP)))
            slot = jnp.where(b == 1, N_RES + _ring(p), _a_slot(p))
            q = _head(qt_s, h, n)
            m = lax.fori_loop(0, NK, lambda t, m: jnp.maximum(m, jnp.max(scores(q, t), axis=0, keepdims=True)),
                              jnp.full((1, BQ), -jnp.inf, F32))
            m_s[h, :, _span(n, BQ)] = m

            def step(t, acc):
                e = jnp.exp2(scores(q, t) - m)
                p_put(slot, t, e[KV:])
                return (acc[0] + _dot(_ld(kvt_s, slice(8, 16), _span(t, KC)), e.astype(BF16)),
                        acc[1] + jnp.sum(e, axis=0, keepdims=True))

            o, l = lax.fori_loop(0, NK, step, (jnp.zeros((DH, BQ), F32), jnp.zeros((1, BQ), F32)))
            l_s[h, :, _span(n, BQ)] = 1.0 / l
            _set_head(ot_s, h, n, o * (1.0 / l))
            pl.when(jnp.logical_and(b == 1, p < NP - 1))(lambda: _start(p_store(p)))
            return carry

        for p in range(NP - N_RING, NP - 1):
            _wait(p_store(p))
        lax.fori_loop(0, 2 * NP, block, 0)

    def middle(act_s, du_s, col_s, row_s, sem, w_sem):
        last = len(F_CHUNKS) - 1

        def w_piece(i, m, j):
            page, row = divmod(((i % 3 * 2 + m) * NS + j) * FC, 512)
            return N_RES * PAGES + page, pl.ds(row, F_CHUNKS[i][1])

        def w_copies(i, out=False):
            return _copies([(w.at[pl.ds(*F_CHUNKS[i]), pl.ds(j * 128, 128)], p_s.at[w_piece(i, m, j)])
                            for m, w in enumerate((dw1t_hbm, dw2_hbm) if out else (w1t_hbm, w2_hbm))
                            for j in range(NS)], w_sem.at[i % 3], out)

        def wc_slot(i, m):
            return 2 * (i & 1) + m

        def wc_piece(i, m, j, f):
            return (N_RES + wc_slot(i, m)) * PAGES + 3 * j + f // 512, pl.ds(0, min(512, F - f))

        def wc_in(i, m):
            return [((w1t_hbm, w2_hbm)[m].at[pl.ds(f, min(512, F - f)), _span(4 * i + j, 128)],
                     p_s.at[wc_piece(i, m, j, f)], p_sem.at[wc_slot(i, m)])
                    for j in range(LT) for f in range(0, F, 512)]

        def gate_b():
            x = q32_s[...].reshape(128, D)
            return jnp.concatenate([x[:, _lanes(d)] for d in range(ND)], axis=0)

        def hidden():
            _wait(biases + p_store(NP - N_RING) + p_store(NP - N_RING + 1))
            _start(w_copies(0))
            pace = _Pacer(never())
            col_s[0] = _col(mod(2))
            col_s[1] = _col(mod(3))
            col_s[2] = _col(1.0 + mod(4))
            gb = _col(mod(5))
            q32_s[...] = jnp.concatenate([gb[_lanes(d)] for d in range(ND)], axis=1).reshape(q32_s.shape)

            def normalize(s, x1):
                mean2 = _mean(x1)
                rstd2 = yield from _rstd(8, lambda rows, words: x1[rows] - pace.now(mean2, rows))
                h2 = []

                def modulate(rows, words):
                    h2.append((x1[rows] - mean2) * pace.now(rstd2, rows) * col_s[2, rows] + col_s[1, rows])
                    return h2[-1:]

                mean3, = yield from _means(8, modulate)
                h2 = jnp.concatenate(h2, axis=0)
                rstd3 = yield from _rstd(8, lambda rows, words: h2[rows] - pace.now(mean3, rows))
                for j, stat in enumerate((mean2, rstd2, mean3, rstd3)):
                    st_s[2 + j, :, _lanes(s)] = stat
                for rows, words in _row_groups(8):
                    h_s[s, words] = _pk((h2[rows] - mean3) * pace.now(rstd3, rows))
                    yield

            for s in range(NS):
                x1 = _ld(xt_s, s).astype(F32) + col_s[0] * pace.dot(_words(_get(wo_s, 0, ALL)), ot_s[s])
                xt_s[s] = _pk(x1)
                pace.add(normalize(s, x1), 32, 0.12, 1.7)
            pace.drain()
            row_s[1] = b2_s[...].astype(F32).reshape(1, S)
            row_s[0, :, 0:F] = b1_s[...].astype(F32).reshape(1, F)

            def h3():
                return pltpu.bitcast(_strips(h_s, 0, NS), BF16)

            for i, (f0, n) in enumerate(F_CHUNKS):
                _wait(w_copies(i))
                if i == 0:
                    _wait(p_store(NP - N_RING + 2) + p_store(NP - N_RING + 3))
                    _start(square_copies(wo_hbm, sem.at[1]))
                if i >= 2:
                    _wait(w_copies(i - 2, out=True))
                _start(w_copies(i + 1) if i < last else wc_in(0, 0))
                w1t, w2 = (jnp.concatenate([p_s[w_piece(i, m, j)] for j in range(NS)], axis=1) for m in range(2))
                gb = jnp.concatenate([gate_b()] * (FC // 128), axis=1)[:, :n]
                if n == FC:
                    u, dact = _dot_nt(h3(), w1t), _dot_nt(_ld(gt_s, ALL, ALL), w2)
                else:
                    u, dact = _dot_nt(w1t, h3()).T, _dot_nt(w2, _ld(gt_s, ALL, ALL)).T
                act, grad = _gelu_and_grad(u + row_s[0, :, f0:f0 + n])
                du = dact * (gb * grad)
                row_s[0, :, f0:f0 + n] = jnp.sum(du, axis=0, keepdims=True)
                act_s[:, f0:f0 + n] = _pk(act)
                du_s[:, f0:f0 + n] = _pk(du)
                if i == last:
                    _wait(w_copies(i - 1, out=True))
                    _start(wc_in(0, 1))
                db2 = []
                for m, lhs in ((1, act * gb), (0, du)):
                    dw = _dot(lhs.astype(BF16).T, _ld(gt_s, ALL, ALL) if m else h3())
                    for j in range(NS):
                        p_s[w_piece(i, m, j)] = dw[:, _lanes(j)].astype(BF16)
                        if i == 1 and m == 0:
                            pace.gate = dw[-8:, _lanes(j)]
                            dy = gate_b() * pace.now(1.0, slice(0, D)) * _ld(gt_s, ALL, _lanes(j)).astype(F32)
                            db2.append(jnp.sum(dy, axis=0, keepdims=True))
                        if j % 4 == 3:
                            _start(w_copies(i, out=True)[m * NS + j - 3:m * NS + j + 1])
                if i == 1:
                    b2_s[...] = jnp.concatenate(db2, axis=1).reshape(S).astype(BF16)
            b1_s[...] = row_s[0, :, 0:F].reshape(F).astype(BF16)
            _start(bias_grads)

        hidden()

        def tokens(out_buf):
            def out_copies(i):
                return token_copies(out_hbm, i, out_buf, 0, sem.at[0], out=True)

            h_s[0:14] = jnp.zeros((14, D // 2, 128), U32)
            _wait(square_copies(wo_hbm, sem.at[1]))

            def chunk(i, carry):
                pl.when(i + 1 == n_tc)(lambda: _start(p_load(NI - 1, 2) + p_load(NI - 1, 1)))
                _wait(wc_in(i, 0) + wc_in(i, 1))
                pace = _Pacer(never())
                da, dx1, outs, do = {}, {}, [], []

                def times(words_ref, m, j):
                    parts = [pace.dot(words_ref[:, f:min(f + 512, F)], p_s[wc_piece(i, m, j, f)])
                             for f in range(0, F, 512)]
                    return functools.reduce(jnp.add, parts)

                def back(j, dh3):
                    t = _span(4 * i + j, 128)
                    mean2, rstd2, mean3, rstd3 = (st_s[2 + n, :, t] for n in range(4))
                    n2 = (_ld(xt_s, 4 * i + j).astype(F32) - mean2) * rstd2
                    h3 = (n2 * col_s[2] + col_s[1] - mean3) * rstd3
                    a1, a2 = _mean(dh3), _mean(dh3 * h3)
                    dn2 = []

                    def sums(rows, words):
                        dh2 = (dh3[rows] - pace.now(a1, rows) - h3[rows] * pace.now(a2, rows)) * rstd3
                        acc_add(4, dh2, rows)
                        acc_add(5, dh2 * n2[rows], rows)
                        dn2.append(dh2 * col_s[2, rows])
                        return [dn2[-1], dn2[-1] * n2[rows]]

                    b1, b2 = yield from _means(4, sums)
                    yield
                    pieces = []
                    for (rows, words), dn in zip(_row_groups(4), dn2):
                        val = (dn - pace.now(b1, rows) - n2[rows] * pace.now(b2, rows)) * rstd2
                        val = _ld(gt_s, words, t).astype(F32) + val
                        pieces.append((col_s[0, rows] * val, val))
                        yield
                    da[j], dx1[j] = (jnp.concatenate(x, axis=0).astype(BF16) for x in zip(*pieces))

                pace.add(back(0, times(du_s, 0, 0)), 33, 0.3, 2.9)
                for j in range(LT):
                    t = _span(4 * i + j, 128)
                    if j + 1 < LT:
                        pace.add(back(j + 1, times(du_s, 0, j + 1)), 33, 0.3, 2.9)
                    else:
                        pl.when(i + 1 == n_tc)(lambda: _start(p_load(NI - 1, 0)))
                    if j == 1:
                        pl.when(i > 0)(lambda: _wait(out_copies(i - 1)))
                        pl.when(i == 0)(lambda: _wait(w_copies(last, out=True)))
                        pl.when(i + 1 < n_tc)(lambda: _start(wc_in(i + 1, 0) + wc_in(i + 1, 1)))
                    y = times(act_s, 1, j) + row_s[1, :, t]
                    acc_add(6, _ld(gt_s, ALL, t).astype(F32) * y)
                    outs.append((j, _ld(xt_s, 4 * i + j).astype(F32) + gate_b() * y))
                    while j and outs:
                        u, out = outs.pop(0)
                        for d in range(ND):
                            out_buf[d, _lanes(u), :] = out[_lanes(d)].T.astype(BF16)
                    do.append(_dot(_get(wo_s, 0, ALL), da[j]).reshape(H, DH, 128) * l_s[:, :, t])
                    l_s[:, :, t] = jnp.sum(do[j] * ot_s[4 * i + j].astype(F32).reshape(H, DH, 128),
                                           axis=1, keepdims=True)
                _start(out_copies(i))
                for j in range(LT):
                    gt_s[:, _span(4 * i + j, 128)] = _words(dx1[j])
                for j in range(ND):
                    pace.add(_fill_table(xt_s, k_s, 4 * i + j, DH), 8, 0.1, 0.9, ahead=True)
                    acc_add(j, pace.dot(_words(_strips(ot_s, 4 * i, LT)),
                                        _ld(gt_s, _span(j, 64), _span(i, TC)), _dot_nt))
                pace.drain()
                for j in range(LT):
                    ot_s[4 * i + j] = do[j].reshape(D, 128).astype(BF16)
                return carry

            lax.fori_loop(0, n_tc, chunk, 0)
            for j in range(ND):
                z, cols = acc_get(j), _lanes(2 * ND + j)
                dmod_s[:, cols] = jnp.sum(wo_s[0, j].astype(F32) * z, axis=0, keepdims=True)
                wo_s[0, j] = (z * mod_s[:, cols]).astype(BF16)
            _start(square_copies(dwo_hbm, b_sem.at[2], out=True))
            for j in range(3):
                dmod_s[:, (3 + j) * D:(4 + j) * D] = _row_total(acc_get(4 + j))
            _wait(out_copies(n_tc - 1))

        pl.run_scoped(tokens, pltpu.VMEM((ND, TC, 128), BF16))

    pl.run_scoped(middle, pltpu.VMEM((D // 2, F), U32), pltpu.VMEM((D // 2, F), U32),
                  pltpu.VMEM((3, D, 128), F32), pltpu.VMEM((2, 1, S), F32), pltpu.SemaphoreType.DMA((2,)),
                  pltpu.SemaphoreType.DMA((3,)))

    def backward(wmod_buf, v_s, dkv_s, col_s, sem):
        x_slot = 2 * UP + 1
        x_in = [staged(x_hbm, i, x_slot, g_sem.at[i]) for i in range(n_tc)]
        dx_out = [staged(dx_hbm, i, x_slot, g_sem.at[i], out=True) for i in range(n_tc)]
        wq_in = square_copies(wq_hbm, sem.at[0])
        wmod_in = [(wmod_hbm.at[:, pl.ds(j * 128, 128)], wmod_buf.at[j], sem.at[1]) for j in range(6 * ND)]
        dkv_s[...] = jnp.zeros(dkv_s.shape, F32)
        lane = lax.broadcasted_iota(jnp.int32, (KC // 2, 128), 1)
        first = lax.broadcasted_iota(jnp.int32, (KC // 2, 128), 0) < KV // 2
        ones = _words(jnp.ones((KC, 128), BF16))
        for t in range(NK):
            kv = k_s[_span(t, KC // 2), :]
            v_s[_span(t, KC // 2), :] = jnp.where(first, jnp.where(lane < DH, kv, 0), jnp.where(
                lane < DH, 0, jnp.where(lane < 2 * DH, kv, jnp.where(lane < 2 * DH + 2, ones, 0))))

        def redo(h, carry):
            slots = [_a_slot(2 * h + k) for k in range(2)]

            @pl.when(no_shift)
            def _():
                for k, slot in enumerate(slots):
                    q = _head(qt_s, h, 2 * k)
                    q32_s[k] = q.astype(F32)
                    for t in range(NK):
                        rows, parts = _vpu_rows(h_s, t, q32_s.at[k], REDO_PARTS)
                        rest = _dot(_mxu_keys(never(), k_s, t, parts)[:, :DH], q)
                        p_put(slot, t, jnp.exp2(jnp.concatenate([rows, rest], axis=0)))

            @pl.when(jnp.logical_not(no_shift))
            def _():
                def step(t, carry):
                    for k, slot in enumerate(slots):
                        s = scores(_head(qt_s, h, 2 * k), t) - m_s[h, :, _span(2 * k, BQ)]
                        p_put(slot, t, jnp.exp2(s)[KV:])
                    return carry

                lax.fori_loop(0, NK, step, 0)

            return carry

        def use(st, t, ds, mask=None, parts=(None,) * 3):
            _, q, do, slot, h, n = st
            do, q, kt = (pltpu.bitcast(_after(mask, w, part), BF16)
                         for w, part in zip((_words(do), _words(q), kvt_s[0:8, _lanes(t)]), parts))
            e = jnp.concatenate([p_s[p_tile(slot, t, j)].reshape(KM, 128) for j in range(LT)], axis=1)
            e = jnp.concatenate([_get(top_s, t % 4, ALL), e], axis=0)
            dkv_s[DH:2 * DH, _lanes(t)] += _dot_nt(do, e)
            dkv_s[0:DH, _lanes(t)] += _dot_nt(q, ds)
            st[0] = st[0] + _dot(kt, ds)
            if t == NK - 1:
                _set_head(ot_s, h, n, st[0] * DH ** -0.5)

        def tail(i, dq, real=True):
            h = i * (UP // 2)
            do = jnp.where(real, _head(ot_s, h, 0).astype(F32), 0.0).astype(BF16)
            return carried([dq, _head(qt_s, h, 0), do, _a_slot(i * UP), h, jnp.where(real, 0, 1)])

        def heads(r, dq_prev):
            i = NI - 1 - r

            @pl.when(jnp.logical_or(i * UP < REDO_A, i < 2))
            def _():
                @pl.when(i == 1)
                def _():
                    _wait(square_copies(dwo_hbm, b_sem.at[2], out=True))
                    _start(wq_in + sum(x_in, []))

                pl.when(i == 0)(lambda: _start(wmod_in))
                lax.fori_loop(i * (UP // 2), jnp.minimum((i + 1) * (UP // 2), REDO_A // 2), redo, 0)

            _wait(sum((p_load(i, k) for k in range(UP - 1)), []))
            pl.when(r > 0)(lambda: _wait(p_load(i, UP - 1)))
            for u in range(2):
                list(_fill_table(h_s, k_s, (2 * r + u) & (NK - 1), 0, KV))
            mask = never()
            row = lax.broadcasted_iota(jnp.int32, (DH, BQ), 0)
            blocks = []
            for j, p, h, n, _ in sorted(_blocks(i), key=lambda blk: (-blk[4], -blk[0])):
                do, c = _head(ot_s, h, n), _span(n, BQ)
                q32_s[j] = do.astype(F32)
                blocks.append((j, p, h, n, _head(qt_s, h, n), do, -l_s[h, :, c], m_s[h, :, c]))
            pending = tail(jnp.minimum(i + 1, NI - 1), dq_prev, r > 0)
            for (j, p, h, n, q, do, shift, m), before in zip(blocks, [(0,)] + blocks):
                slot = N_RES + _ring_back(j // 2) if j % 2 else _a_slot(p)
                if j == 2 * UP - 1:
                    slot = jnp.where(r > 0, slot, N_RES + N_RING - 1)
                high = shift.astype(BF16).astype(F32)
                extra = jnp.where(row == 0, high, jnp.where(row == 1, shift - high, 0.0)).astype(BF16)
                rhs = jnp.concatenate([q, do, extra], axis=0)
                shift = [jnp.broadcast_to(shift[:, _lanes(u)], (1, 1, 8, 128)) for u in range(LT)]
                st = [jnp.zeros((DH, BQ), F32), q, do, slot, h, n]
                for t in range(NK):
                    rows, parts = _vpu_rows(xt_s, t, q32_s.at[j], BWD_PARTS, shift)
                    out = _dot(_mxu_keys(mask, v_s, t, parts[:8])[:, :3 * DH], rhs)
                    top = jnp.exp2(out[:KV] - m)
                    rest = jnp.concatenate([p_s[p_tile(slot, t, u)].astype(F32).reshape(KM, 128)
                                            for u in range(LT)], axis=1)
                    ds = jnp.concatenate([rows * top, out[KV:] * rest], axis=0)
                    _put(top_s, t % 4, ALL, top)
                    if j == 0 and t >= NK - LAG:
                        _put(lag_s, t - (NK - LAG), ALL, ds)
                    else:
                        pending.append((st, t, ds.astype(BF16)))
                    use(*pending.pop(0), mask, parts[8:])
                    if before[0] % 2 and t == LAG - 1:
                        pl.when(i > 0)(lambda k=before[0] // 2: _start(p_load(i - 1, k)))
            return st[0]

        lag_s[...] = jnp.zeros(lag_s.shape, BF16)
        top_s[...] = jnp.zeros(top_s.shape, BF16)
        for item in tail(0, lax.fori_loop(0, NI, heads, jnp.zeros((DH, BQ), F32))):
            use(*item)

        def epilogue():
            def dwmod_part(lo, hi):
                for j in range(lo, hi):
                    for r in range(ND):
                        part = col_s[2, _lanes(r)] * pace.now(dmod_s[:, _lanes(j)], _lanes(r))
                        wmod_buf[j, _lanes(r), :] = part.astype(BF16)
                        yield
                _start(dwmod_out[lo:hi])

            def finish(s, dh1):
                rstd = st_s[1, :, _lanes(s)]
                n1 = (_ld(xt_s, s).astype(F32) - st_s[0, :, _lanes(s)]) * rstd
                qt_s[s] = (n1 * col_s[1] + col_s[0]).astype(BF16)
                (acc_add if s else acc_set)(4, dh1)
                (acc_add if s else acc_set)(5, dh1 * n1)
                dn1 = dh1 * col_s[1]
                a1, a2 = _mean(dn1), _mean(dn1 * n1)
                yield
                for d in range(ND):
                    dx = []
                    for rows, words in _row_groups(4)[4 * d:4 * d + 4]:
                        val = (dn1[rows] - pace.now(a1, rows) - n1[rows] * pace.now(a2, rows)) * rstd
                        dx.append(_ld(gt_s, words, _lanes(s)).astype(F32) + val)
                        yield
                    p_s[staged_tile(x_slot, s, d)] = jnp.concatenate(dx, axis=0).T.astype(BF16)
                if s % 4 == 3:
                    _start(dx_out[s // 4])

            def transpose(s):
                for r in _row_groups(16):
                    yield _words(transpose_x(x_slot, s, *r))[-8:]

            def dsilu_part(j):
                return _dot_nt(jnp.broadcast_to(dmod_s[:, _lanes(j)].astype(BF16), (16, 128)), wmod_buf[j])

            def dw_part(s):
                i, j = divmod(s, LT)
                part = pace.dot(_words(_strips(qt_s, 4 * i, LT)), _strips(ot_s, 4 * i, LT, _lanes(j)), _dot_nt)
                if i:
                    part += acc_get(j)
                if i + 1 < n_tc:
                    acc_set(j, part)
                else:
                    wo_s[0, j] = part.astype(BF16)
                    _start(dwq_out[j:j + 1])
                return _dot_nt(dkv[:, _lanes(s)], qt_s[s])

            _wait(wq_in + wmod_in + sum(x_in[:3], []))
            pace = _Pacer(never())
            col_s[0] = _col(mod(0))
            col_s[1] = _col(1.0 + mod(1))
            col_s[2] = _col(silu_c().astype(F32))
            wkv = jnp.concatenate([wkv_s[...], jnp.zeros((128 - 2 * DH, D), BF16)], axis=0).T[:, :2 * DH]
            dkv = jnp.concatenate([dkv_s[0:DH] * (1.0 / LOG2E), dkv_s[DH:2 * DH]], axis=0).astype(BF16)
            dsilu, dwkv = jnp.zeros((16, D), F32), jnp.zeros((2 * DH, D), F32)
            dwq_out = square_copies(dwq_hbm, sem.at[0], out=True)
            dwmod_out = [(wmod_buf.at[j], dwmod_hbm.at[:, pl.ds(j * 128, 128)], sem.at[1]) for j in range(6 * ND)]

            list(transpose(0))
            waits = {8: x_in[3], 13: dx_out[0], 17: dx_out[1]}
            dw_steps = [s for s in range(LT, NS + LT + 2) if s not in (9, 13)]
            outer = {5: (8, 10), 7: (10, 12), 9: (12, 15), 11: (15, 18), 13: (18, 21), 15: (21, 24)}
            for s in range(dw_steps[-1] + 1):
                _wait(waits.get(s, []))
                if s < NS:
                    dsilu += dsilu_part(2 * ND + s)
                    if s + 1 < NS:
                        pace.add(transpose(s + 1), 4, 0.4, 1.0, ahead=True)
                    job = finish(s, pace.dot(_words(_get(wo_s, 0, ALL)), ot_s[s]) + _dot(wkv, dkv[:, _lanes(s)]))
                    next(job)
                    pace.add(job, 16, 0.15, 1.9)
                if s in outer:
                    pace.add(dwmod_part(*outer[s]), 12, 0.0, 2.9 if s < NS - 1 else 0.9)
                if s == NS - 1:
                    dmod_s[:, 0:D] = _row_total(acc_get(4))
                    dmod_s[:, D:2 * D] = _row_total(acc_get(5))
                if s in dw_steps:
                    dwkv += dw_part(dw_steps.index(s))
                if s in (NS, NS + 1):
                    dsilu += sum(dsilu_part(ND * (s - NS) + j) for j in range(ND))
                    pace.add(dwmod_part(ND * (s - NS), ND * (s - NS + 1)), 16, 0.05, 0.85)
            pace.drain()
            wkv_s[...] = dwkv.astype(BF16)
            c_in = c_s[...].astype(F32)
            sig_c = jax.nn.sigmoid(c_in)
            c_s[...] = (dsilu[0:1] * (sig_c * (1.0 + c_in * (1.0 - sig_c)))).astype(BF16)
            small = [(wkv_s.at[pl.ds(0, DH)], dwkt_hbm, sem.at[0]), (wkv_s.at[pl.ds(DH, DH)], dwvt_hbm, sem.at[0]),
                     (c_s, dc_hbm, sem.at[0])]
            _start(small)
            _wait(dwmod_out + dx_out[2] + dx_out[3] + small + dwq_out + bias_grads)

        epilogue()

    pl.run_scoped(backward, pltpu.VMEM((6 * ND, D, 128), BF16), pltpu.VMEM((S // 2, 128), U32),
                  pltpu.VMEM((2 * DH, S), F32), pltpu.VMEM((3, D, 128), F32), pltpu.SemaphoreType.DMA((2,)))


@jax.jit
def pallas_adaLN_cond__grouped_kv_mqa__mixer_token_mlp__prompt_kernel(
    A_x: jax.Array,
    A_wq: jax.Array,
    A_wk: jax.Array,
    A_wv: jax.Array,
    A_wo: jax.Array,
    B_x: jax.Array,
    B_w1: jax.Array,
    B_b1: jax.Array,
    B_w2: jax.Array,
    B_b2: jax.Array,
    c: jax.Array,
    w_mod: jax.Array,
    grad_out: jax.Array,
):
    del B_x
    hbm = pl.BlockSpec(memory_space=pl.ANY)
    sds = jax.ShapeDtypeStruct
    outs = pl.pallas_call(
        _kernel,
        in_specs=[hbm] * 12,
        out_specs=[hbm] * 13,
        out_shape=[
            sds((1, S, D), BF16), sds((1, S, D), BF16), sds((D, D), BF16), sds((DH, D), BF16),
            sds((DH, D), BF16), sds((D, D), BF16), sds((F, S), BF16), sds((F,), BF16), sds((F, S), BF16),
            sds((S,), BF16), sds((1, D), BF16), sds((D, 6 * D), BF16),
            sds((NP - 1, PAGES, 512, 128), BF16),
        ],
        scratch_shapes=[
            pltpu.VMEM(((N_RES + N_RING) * PAGES, 512, 128), BF16),
            pltpu.VMEM((NS, D // 2, 128), U32),
            pltpu.VMEM((NS, D, 128), BF16),
            pltpu.VMEM((NS, D, 128), BF16),
            pltpu.VMEM((D // 2, S), U32),
            pltpu.VMEM((NS, D // 2, 128), U32),
            pltpu.VMEM((S // 2, 128), U32),
            pltpu.VMEM((DH, S), U32),
            pltpu.VMEM((1, ND, D, 128), BF16),
            pltpu.VMEM((2 * DH, D), BF16),
            pltpu.VMEM((F,), BF16),
            pltpu.VMEM((S,), BF16),
            pltpu.VMEM((1, D), BF16),
            pltpu.VMEM((H, 1, S), F32),
            pltpu.VMEM((H, 1, S), F32),
            pltpu.VMEM((1, 6 * D), F32),
            pltpu.VMEM((1, 6 * D), F32),
            pltpu.VMEM((6, 1, S), F32),
            pltpu.VMEM((2 * UP, DH, BQ), F32),
            pltpu.VMEM((LAG, LT, KC, 128), BF16),
            pltpu.VMEM((4, LT, KV, 128), BF16),
            pltpu.VMEM((8, 128), F32),
            pltpu.SemaphoreType.DMA((N_RING,)),
            pltpu.SemaphoreType.DMA((3,)),
            pltpu.SemaphoreType.DMA((S // TC,)),
        ],
        compiler_params=pltpu.CompilerParams(vmem_limit_bytes=128 * 1024 * 1024),
        name="adaln_mqa_mixer_fwd_bwd",
    )(A_x, A_wq, A_wk.T, A_wv.T, A_wo, B_w1.T, B_b1, B_w2, B_b2, c, w_mod, grad_out)
    out, dx, dwq, dwkt, dwvt, dwo, dw1t, db1, dw2, db2, dc, dwmod, _ = outs
    return out, dx, dwq, dwkt.T, dwvt.T, dwo, dw1t.T, db1, dw2, db2, dc, dwmod
```
